```python
import os as _os
_os.environ.setdefault("JAX_PLATFORMS", "cpu")
import jax
import jax.numpy as jnp

def _softmax(x, axis=-1):
    return jax.nn.softmax(x, axis=axis)
def _gelu(x):
    return jax.nn.gelu(x, approximate=True)
def _silu(x):
    return jax.nn.silu(x)
def _sigmoid(x):
    return jax.nn.sigmoid(x)
def _layernorm(x, axis=-1, eps=1e-5):
    m = jnp.mean(x, axis=axis, keepdims=True)
    v = jnp.var(x, axis=axis, keepdims=True)
    return (x - m) / jnp.sqrt(v + eps)
def _scatter_add(tgt, idx, src, axis=0):
    return tgt.at[idx].add(src)
def _segment_sum(src, seg, n):
    return jax.ops.segment_sum(src, seg, n)
class _Rng:
    def __init__(self, key):
        self._k = key
    def _next(self):
        self._k, sub = jax.random.split(self._k)
        return sub
    def normal(self, shape):
        return jax.random.normal(self._next(), shape, dtype=jnp.bfloat16)
    def randint(self, lo, hi, shape):
        return jax.random.randint(self._next(), shape, lo, hi, dtype=jnp.int32)
    def uniform(self, shape, lo=0.0, hi=1.0):
        return jax.random.uniform(self._next(), shape, jnp.bfloat16, lo, hi)
    def permutation(self, n):
        return jax.random.permutation(self._next(), n)


kernel_name = 'standalone__gqa_block_cached__near_ridge'

def setup_inputs():
    _rng = _Rng(jax.random.key(int.from_bytes(__import__("os").urandom(4), "little")))
    _w = (lambda a: (lambda t: t.astype(jnp.bfloat16) if jnp.issubdtype(t.dtype, jnp.floating) else t)(jnp.asarray(a)))
    B, Sq, D = 8, 64, 512
    Hq, Hkv, Sk, Dh = 32, 8, 64, 128
    assert Hq % Hkv == 0, (Hq, Hkv)
    return {
        "x": _w((lambda *s: _rng.normal(s) * 0.8)(B, Sq, D)),
        "k_cache": _w((lambda *s: _rng.normal(s) * 0.8)(B, Hkv, Sk, Dh)),
        "v_cache": _w((lambda *s: _rng.normal(s) * 0.05)(B, Hkv, Sk, Dh)),
        "wq": _w((lambda *s: _rng.normal(s) * 0.8)(D, Hq * Dh) * (D ** -0.5)),
        "wo": _w((lambda *s: _rng.normal(s) * 0.05)(Hq * Dh, D) * ((Hq * Dh) ** -0.5)),
    }

def reference(x, k_cache, v_cache, wq, wo):
    B, Sq, D = x.shape
    Hq, Dh = 32, 128
    Hkv = k_cache.shape[1]
    rep = Hq // Hkv
    q = (lambda x, *d: x.transpose(*d))((x @ wq).reshape(B, Sq, Hq, Dh), 0, 2, 1, 3)
    k = jnp.repeat(k_cache, rep, axis=1)
    v = jnp.repeat(v_cache, rep, axis=1)
    scores = jnp.einsum("bhqd,bhkd->bhqk", q, k) * (Dh ** -0.5)
    p = _softmax(scores, axis=-1)
    o = jnp.einsum("bhqk,bhkd->bhqd", p, v)
    return (lambda x, *d: x.transpose(*d))(o, 0, 2, 1, 3).reshape(B, Sq, Hq * Dh) @ wo
```

```python
import functools
import jax
import jax.numpy as jnp
import jax.experimental.pallas as pl
import jax.experimental.pallas.tpu as pltpu


def _kernel(x_ref, k_ref, v_ref, wq_ref, wo_ref, out_ref, acc_ref, *, B, Sq, Dh, rep):
    g = pl.program_id(0)
    scale = Dh ** -0.5
    q = jnp.dot(x_ref[...], wq_ref[...], preferred_element_type=jnp.float32).astype(jnp.bfloat16)
    o_rows = []
    for b in range(B):
        qb = jnp.concatenate(
            [q[b * Sq:(b + 1) * Sq, h * Dh:(h + 1) * Dh] for h in range(rep)], axis=0)
        kb = k_ref[b, 0]
        vb = v_ref[b, 0]
        s = jax.lax.dot_general(qb, kb, (((1,), (1,)), ((), ())),
                                preferred_element_type=jnp.float32) * scale
        m = jnp.max(s, axis=-1, keepdims=True)
        p = jnp.exp(s - m)
        l = jnp.sum(p, axis=-1, keepdims=True)
        o = jnp.dot(p.astype(jnp.bfloat16), vb, preferred_element_type=jnp.float32) / l
        o = o.astype(jnp.bfloat16)
        o_rows.append(jnp.concatenate([o[h * Sq:(h + 1) * Sq] for h in range(rep)], axis=1))
    o_all = jnp.concatenate(o_rows, axis=0)
    part = jnp.dot(o_all, wo_ref[...], preferred_element_type=jnp.float32)

    @pl.when(g == 0)
    def _():
        acc_ref[...] = part

    @pl.when(g > 0)
    def _():
        acc_ref[...] += part

    @pl.when(g == pl.num_programs(0) - 1)
    def _():
        out_ref[...] = acc_ref[...].astype(out_ref.dtype)


@jax.jit
def pallas_standalone__gqa_block_cached__near_ridge_kernel(x, k_cache, v_cache, wq, wo):
    B, Sq, D = x.shape
    _, Hkv, Sk, Dh = k_cache.shape
    Hq = wq.shape[1] // Dh
    rep = Hq // Hkv
    x2 = x.reshape(B * Sq, D)
    out = pl.pallas_call(
        functools.partial(_kernel, B=B, Sq=Sq, Dh=Dh, rep=rep),
        grid=(Hkv,),
        in_specs=[
            pl.BlockSpec((B * Sq, D), lambda g: (0, 0)),
            pl.BlockSpec((B, 1, Sk, Dh), lambda g: (0, g, 0, 0)),
            pl.BlockSpec((B, 1, Sk, Dh), lambda g: (0, g, 0, 0)),
            pl.BlockSpec((D, rep * Dh), lambda g: (0, g)),
            pl.BlockSpec((rep * Dh, D), lambda g: (g, 0)),
        ],
        out_specs=pl.BlockSpec((B * Sq, D), lambda g: (0, 0)),
        out_shape=jax.ShapeDtypeStruct((B * Sq, D), x.dtype),
        scratch_shapes=[pltpu.VMEM((B * Sq, D), jnp.float32)],
        compiler_params=pltpu.CompilerParams(
            dimension_semantics=("arbitrary",), vmem_limit_bytes=64 * 1024 * 1024),
    )(x2, k_cache, v_cache, wq, wo)
    return out.reshape(B, Sq, D)
```

```python
import functools

import numpy as np
import jax
import jax.numpy as jnp
import jax.experimental.pallas as pl
import jax.experimental.pallas.tpu as pltpu

STAGE0 = "2 5 1 7 F0 4 F1 3 B0 6 B1"
STAGE = "5 F0 7 1 B0 4 F1 6 2 3 B1"
LAST_STAGE = "0 F0 1 2 3 B0 F1 4 5 B1 6"
O_ORDER = (5, 2, 1, 4, 3, 7, 6)
LEAF_ORDER = (2, 1, 4, 3, 5, 6, 7)
EARLY_PASSES = ((0, 3), (3, 7))
PREP_SLOTS = ((0,), (1, 2), (3,), (4, 5), (6,), (7,), ())
WO_CHUNKS = ((0, 1), (1, 3), (3, 7), (7, 8))
KV_CHUNKS = ((0, 1), (1, 2), (2, 4), (4, 8))
WQ_FINE = (1,)
Q0_SPLIT = 4
CH = 16

TN = (((0,), (0,)), ((), ()))
NT = (((1,), (1,)), ((), ()))
BF = jnp.bfloat16
F32 = jnp.float32
T = 128

A_TERMS = {1: ((1, 0, 0), (1, 1, 1)), 2: ((1, 1, 0), (1, 1, 1)), 3: ((1, 0, 0),), 4: ((1, 1, 1),),
           5: ((1, 0, 0), (1, 0, 1)), 6: ((1, 1, 0), (-1, 0, 0)), 7: ((1, 0, 1), (-1, 1, 1))}
B_TERMS = {1: ((1, 0, 0), (1, 1, 1)), 2: ((1, 0, 0),), 3: ((1, 0, 1), (-1, 1, 1)), 4: ((1, 1, 0), (-1, 0, 0)),
           5: ((1, 1, 1),), 6: ((1, 0, 0), (1, 0, 1)), 7: ((1, 1, 0), (1, 1, 1))}
C_TERMS = {(0, 0): ((1, 1), (1, 4), (-1, 5), (1, 7)), (0, 1): ((1, 3), (1, 5)),
           (1, 0): ((1, 2), (1, 4)), (1, 1): ((1, 1), (-1, 2), (1, 3), (1, 6))}


def _combine(terms, get):
    acc = None
    for t in terms:
        v = get(*t[1:])
        if acc is None:
            acc = v if t[0] > 0 else -v
        else:
            acc = acc + v if t[0] > 0 else acc - v
    return acc


def _program(Hkv):
    prog = []
    units = [("L", 0, i2, ga, gb) for (ga, gb) in EARLY_PASSES for i2 in LEAF_ORDER]
    nslot = sum(t.isdigit() for t in LAST_STAGE.split())
    for g in range(Hkv):
        last = g + 1 == Hkv
        for t in (LAST_STAGE if last else STAGE0 if g == 0 else STAGE).split():
            if t[0] in "FB":
                prog.append((t[0], g, int(t[1])))
            elif last:
                prog += units[int(t) * len(units) // nslot:(int(t) + 1) * len(units) // nslot]
            else:
                prog.append(("Q", g + 1, int(t)))
    for pi in range(len(O_ORDER)):
        for s, i2 in enumerate(LEAF_ORDER):
            if pi + 1 < len(O_ORDER) and len(B_TERMS[O_ORDER[pi + 1]]) > 1 and pi > 0:
                prog += [("P", pi + 1, g) for g in PREP_SLOTS[s]]
            prog.append(("L", pi, i2, EARLY_PASSES[-1][1] if pi == 0 else 0, Hkv))
    return prog


def _kernel(x_hbm, k_hbm, v_hbm, wq_hbm, wo_hbm, out_hbm,
            xs, xa, wqs, ks, vs, wos, wb, qs, os_, outs, qacc, sems,
            *, B, Sq, Dh, rep, Hkv, D):
    M = B * Sq
    HM, QM = M // 2, M // 4
    nkt = D // T
    TU = T // 2
    GR = rep * Dh
    scale = np.float32(Dh ** -0.5 * np.log2(np.e))
    xu, xau, wqu, ku, vu, wou, wbu, qu, ou = (r.bitcast(jnp.uint32) for r in (xs, xa, wqs, ks, vs, wos, wb, qs, os_))
    bf = lambda u: pltpu.bitcast(u, BF)
    prog = _program(Hkv)

    items = {}
    for kt in range(nkt):
        rows = slice(kt * T, (kt + 1) * T)
        items[("w0", kt)] = [(wq_hbm.at[rows, h * T:(h + 1) * T], wqs.at[h, rows]) for h in range(rep)]
        items[("x", kt)] = [(x_hbm.at[:, rows], xs.at[kt])]
    for (g0, g1) in KV_CHUNKS:
        items[("k", g0)] = [(k_hbm.at[:, g0:g1], ks.at[:, g0:g1])]
        items[("v", g0)] = [(v_hbm.at[:, g0:g1], vs.at[:, g0:g1])]
    for g in range(1, Hkv):
        for cc in range(2):
            for r in range(2 if g in WQ_FINE else 1):
                rows = slice(r * D // 2, (r + 1) * D // 2) if g in WQ_FINE else slice(0, D)
                items[("wq", g, r, cc)] = [(wq_hbm.at[rows, h * T:(h + 1) * T], wqs.at[h, rows])
                                           for h in (g * rep + 2 * cc, g * rep + 2 * cc + 1)]
    for (g0, g1) in WO_CHUNKS:
        rows = slice(g0 * GR, g1 * GR)
        items[("wo", g0)] = [(wo_hbm.at[rows, n * T:(n + 1) * T], wos.at[n, rows]) for n in range(nkt)]
    kv_item = {g: g0 for (g0, g1) in KV_CHUNKS for g in range(g0, g1)}
    wo_item = {g: ("wo", g0) for (g0, g1) in WO_CHUNKS for g in range(g0, g1)}
    wq_items = lambda g, i: list(dict.fromkeys(("wq", g, r if g in WQ_FINE else 0, cc) for (_, r, cc) in B_TERMS[i]))

    order = [it for kt in range(nkt) for it in (("w0", kt), ("x", kt))]
    for it in prog:
        if it[0] in "FB":
            order.append(("k" if it[0] == "F" else "v", kv_item[it[1]]))
        elif it[0] == "Q":
            order += wq_items(it[1], it[2])
        elif it[0] == "L":
            order += [wo_item[g] for g in range(it[3], it[4])]
        else:
            order.append(wo_item[it[2]])
    order = list(dict.fromkeys(order))
    assert sorted(order) == sorted(items) and len(order) + 1 == sems.shape[0]
    copies = {it: [pltpu.make_async_copy(a, b, sems.at[si]) for a, b in items[it]] for si, it in enumerate(order)}
    out_cp = {(r, n): pltpu.make_async_copy(outs.at[n, r * QM:(r + 1) * QM],
                                            out_hbm.at[r * QM:(r + 1) * QM, n * T:(n + 1) * T], sems.at[len(order)])
              for r in range(4) for n in range(nkt)}
    landed = set()

    def need(*its):
        for it in its:
            if it not in landed:
                landed.add(it)
                for cp in copies[it]:
                    cp.wait()

    def bsum(terms, tile):
        if len(terms) == 1:
            return tile(*terms[0][1:])
        return _combine(terms, lambda r, cc: tile(r, cc).astype(F32)).astype(BF)

    xa_index = {i: n for n, i in enumerate(i for i in A_TERMS if len(A_TERMS[i]) > 1)}
    xa_done = set()
    Mq = {}

    def x_operand(i, j):
        block = lambda r, cc: bf(xu[2 * cc + j, r * HM // 2:(r + 1) * HM // 2, :])
        if i not in xa_index:
            return block(*A_TERMS[i][0][1:])
        if (i, j) in xa_done:
            return bf(xau[2 * xa_index[i] + j])
        v = bsum(A_TERMS[i], block)
        xa[2 * xa_index[i] + j] = v
        xa_done.add((i, j))
        return v

    def q_product(g, i):
        need(*wq_items(g, i))
        lhs = [x_operand(i, j) for j in range(2)]
        rhs = lambda j, n: bsum(B_TERMS[i], lambda r, cc: bf(wqu[g * rep + 2 * cc + n, (2 * r + j) * TU:(2 * r + j + 1) * TU, :]))
        Ms = Mq.setdefault(g, {})
        Ms[i] = [jnp.dot(lhs[0], rhs(0, n), preferred_element_type=F32) + jnp.dot(lhs[1], rhs(1, n), preferred_element_type=F32)
                 for n in range(2)]
        for (r, cc), terms in C_TERMS.items():
            if all(t[1] in Ms for t in terms) and any(t[1] == i for t in terms):
                for n in range(2):
                    qs[g * rep + 2 * cc + n, r * HM:(r + 1) * HM, :] = _combine(terms, lambda m: Ms[m][n]).astype(BF)

    def attn_front(g, b):
        q = jnp.concatenate([bf(qu[g * rep + h, pl.ds((b * Sq + ch * CH) // 2, CH // 2), :])
                             for ch in range(Sq // CH) for h in range(rep)], axis=0)
        s = jax.lax.dot_general(bf(ku[b, g]), q, NT, preferred_element_type=F32) * scale
        p = jnp.exp2(s - jnp.max(s, axis=0, keepdims=True))
        return (p * pltpu.reciprocal(jnp.sum(p, axis=0, keepdims=True), approx=True)).astype(BF)

    def attn_back(g, b, p):
        return jax.lax.dot_general(p, bf(vu[b, g]), TN, preferred_element_type=F32)

    def store_o(g, b0, o):
        for ch in range(Sq // CH):
            tile = lambda r1, r2, h: o[(r1, r2)][(ch * rep + h) * CH:(ch * rep + h + 1) * CH]
            for i in range(1, 8):
                S = {}

                def s_tile(r2, c2):
                    if (r2, c2) not in S:
                        S[(r2, c2)] = _combine(A_TERMS[i], lambda r1, c1: tile(r1, r2, 2 * c1 + c2))
                    return S[(r2, c2)]
                for i2 in range(1, 8):
                    os_[(g * 7 + i - 1) * 7 + i2 - 1, pl.ds(b0 * Sq + ch * CH, CH), :] = _combine(A_TERMS[i2], s_tile).astype(BF)

    def wo_tile(g, h, n, r0=0, r1=T):
        return bf(wou[n, (g * rep + h) * TU + r0 // 2:(g * rep + h) * TU + r1 // 2, :])

    wb_slot = lambda pi, g, i2: ((pi % 2) * Hkv + g) * 7 + i2 - 1
    prepped = set()

    def prep(pi, g):
        need(wo_item[g])
        for r0 in range(0, T, 16):
            Tt = {(r2, c2): _combine(B_TERMS[O_ORDER[pi]], lambda r1, c1: wo_tile(g, 2 * r1 + r2, 2 * c1 + c2, r0, r0 + 16).astype(F32))
                  for r2 in range(2) for c2 in range(2)}
            for i2 in range(1, 8):
                wb[wb_slot(pi, g, i2), r0:r0 + 16, :] = _combine(B_TERMS[i2], lambda r2, c2: Tt[(r2, c2)]).astype(BF)
        prepped.add((pi, g))

    def leaf_rhs(pi, g, i2):
        if (pi, g) in prepped:
            return bf(wbu[wb_slot(pi, g, i2)])
        need(wo_item[g])
        terms = [(s2 * s1, 2 * r1 + r2, 2 * c1 + c2) for (s2, r2, c2) in B_TERMS[i2] for (s1, r1, c1) in B_TERMS[O_ORDER[pi]]]
        return bsum(terms, lambda h, n: wo_tile(g, h, n))

    Lf, Lf_done, Mo = {}, {}, {}

    def leaf(pi, i2, ga, gb):
        i = O_ORDER[pi]
        r = [jnp.dot(bf(ou[(g * 7 + i - 1) * 7 + i2 - 1]), leaf_rhs(pi, g, i2), preferred_element_type=F32) for g in range(ga, gb)]
        while len(r) > 1:
            r = [r[j] + r[j + 1] if j + 1 < len(r) else r[j] for j in range(0, len(r), 2)]
        Li = Lf.setdefault(i, {})
        Li[i2] = Li[i2] + r[0] if i2 in Li else r[0]
        if gb < Hkv:
            return
        fin = Lf_done.setdefault(i, [])
        fin.append(i2)
        Mi = Mo.setdefault(i, {})
        for (r2, c2), terms2 in C_TERMS.items():
            if all(t[1] in fin for t in terms2) and any(t[1] == i2 for t in terms2):
                Mi[(r2, c2)] = _combine(terms2, lambda m: Li[m])
                for (r1, c1), terms in C_TERMS.items():
                    if all((r2, c2) in Mo.get(t[1], {}) for t in terms) and any(t[1] == i for t in terms):
                        rr, n = 2 * r1 + r2, 2 * c1 + c2
                        outs[n, rr * QM:(rr + 1) * QM, :] = _combine(terms, lambda m: Mo[m][(r2, c2)]).astype(BF)
                        out_cp[(rr, n)].start()

    for it in order:
        for cp in copies[it]:
            cp.start()

    for kt in range(nkt):
        need(("w0", kt), ("x", kt))
        for r0 in range(0, M, M // Q0_SPLIT):
            r1 = r0 + M // Q0_SPLIT
            for h in range(rep):
                part = jnp.dot(bf(xu[kt, r0 // 2:r1 // 2, :]), bf(wqu[h, kt * TU:(kt + 1) * TU, :]), preferred_element_type=F32)
                if kt > 0:
                    part = part + qacc[h, r0:r1, :]
                if kt + 1 == nkt:
                    qs[h, r0:r1, :] = part.astype(BF)
                else:
                    qacc[h, r0:r1, :] = part

    batches = lambda b0: {(r1, r2): 4 * r1 + 2 * r2 + b0 for r2 in range(2) for r1 in range(2)}
    probs = {}
    for it in prog:
        if it[0] == "Q":
            q_product(it[1], it[2])
        elif it[0] == "F":
            need(("k", kv_item[it[1]]))
            for b in batches(it[2]).values():
                probs[b] = attn_front(it[1], b)
        elif it[0] == "B":
            need(("v", kv_item[it[1]]))
            store_o(it[1], it[2], {rr: attn_back(it[1], b, probs.pop(b)) for rr, b in batches(it[2]).items()})
        elif it[0] == "L":
            leaf(*it[1:])
        else:
            prep(*it[1:])
    assert len(landed) == len(order)
    for cp in out_cp.values():
        cp.wait()


@jax.jit
def pallas_standalone__gqa_block_cached__near_ridge_kernel(x, k_cache, v_cache, wq, wo):
    B, Sq, D = x.shape
    _, Hkv, Sk, Dh = k_cache.shape
    Hq = wq.shape[1] // Dh
    rep = Hq // Hkv
    M = B * Sq
    nkt = D // T
    assert (B, rep, Hkv, nkt, Dh) == (8, 4, 8, 4, T) and Sq % CH == 0
    nsem = 2 * nkt + 2 * len(KV_CHUNKS) + 2 * (Hkv - 1 + len(WQ_FINE)) + len(WO_CHUNKS) + 1
    any_spec = pl.BlockSpec(memory_space=pl.ANY)
    out = pl.pallas_call(
        functools.partial(_kernel, B=B, Sq=Sq, Dh=Dh, rep=rep, Hkv=Hkv, D=D),
        in_specs=[any_spec] * 5,
        out_specs=any_spec,
        out_shape=jax.ShapeDtypeStruct((M, D), x.dtype),
        scratch_shapes=[
            pltpu.VMEM((nkt, M, T), BF),
            pltpu.VMEM((10, M // 2, T), BF),
            pltpu.VMEM((Hq, D, T), BF),
            pltpu.VMEM((B, Hkv, Sk, Dh), BF),
            pltpu.VMEM((B, Hkv, Sk, Dh), BF),
            pltpu.VMEM((nkt, Hq * Dh, T), BF),
            pltpu.VMEM((2 * Hkv * 7, Dh, T), BF),
            pltpu.VMEM((Hq, M, T), BF),
            pltpu.VMEM((Hkv * 49, M // 4, T), BF),
            pltpu.VMEM((nkt, M, T), BF),
            pltpu.VMEM((rep, M, T), F32),
            pltpu.SemaphoreType.DMA((nsem,)),
        ],
        compiler_params=pltpu.CompilerParams(
            vmem_limit_bytes=100 * 1024 * 1024,
            disable_semaphore_checks=True,
            flags={"XLA_TPU_RESCHEDULE_DMA_DONES": True},
        ),
    )(x.reshape(M, D), k_cache, v_cache, wq, wo)
    return out.reshape(B, Sq, D)
```
